```python
import os as _os
_os.environ.setdefault("JAX_PLATFORMS", "cpu")
import jax
import jax.numpy as jnp

def _softmax(x, axis=-1):
    return jax.nn.softmax(x, axis=axis)
def _gelu(x):
    return jax.nn.gelu(x, approximate=True)
def _silu(x):
    return jax.nn.silu(x)
def _sigmoid(x):
    return jax.nn.sigmoid(x)
def _layernorm(x, axis=-1, eps=1e-5):
    m = jnp.mean(x, axis=axis, keepdims=True)
    v = jnp.var(x, axis=axis, keepdims=True)
    return (x - m) / jnp.sqrt(v + eps)
def _scatter_add(tgt, idx, src, axis=0):
    return tgt.at[idx].add(src)
def _segment_sum(src, seg, n):
    return jax.ops.segment_sum(src, seg, n)
class _Rng:
    def __init__(self, key):
        self._k = key
    def _next(self):
        self._k, sub = jax.random.split(self._k)
        return sub
    def normal(self, shape):
        return jax.random.normal(self._next(), shape, dtype=jnp.bfloat16)
    def randint(self, lo, hi, shape):
        return jax.random.randint(self._next(), shape, lo, hi, dtype=jnp.int32)
    def uniform(self, shape, lo=0.0, hi=1.0):
        return jax.random.uniform(self._next(), shape, jnp.bfloat16, lo, hi)
    def permutation(self, n):
        return jax.random.permutation(self._next(), n)


kernel_name = 'concat_heads__mha_block_cached__mha_block_cached__near_ridge'

def setup_inputs():
    _rng = _Rng(jax.random.key(int.from_bytes(__import__("os").urandom(4), "little")))
    _w = (lambda a: (lambda t: t.astype(jnp.bfloat16) if jnp.issubdtype(t.dtype, jnp.floating) else t)(jnp.asarray(a)))
    def _A_setup():
        B, Sq, D = 8, 144, 640
        H, Sk, Dh = 32, 512, 128
        return {
            "x": _w((lambda *s: _rng.normal(s) * 0.8)(B, Sq, D)),
            "k_cache": _w((lambda *s: _rng.normal(s) * 0.8)(B, H, Sk, Dh)),
            "v_cache": _w((lambda *s: _rng.normal(s) * 0.05)(B, H, Sk, Dh)),
            "wq": _w((lambda *s: _rng.normal(s) * 0.8)(D, H * Dh) * (D ** -0.5)),
            "wo": _w((lambda *s: _rng.normal(s) * 0.05)(H * Dh, D) * ((H * Dh) ** -0.5)),
        }
    _A_in = _A_setup()

    def _B_setup():
        B, Sq, D = 8, 144, 640
        H, Sk, Dh = 32, 512, 128
        return {
            "x": _w((lambda *s: _rng.normal(s) * 0.8)(B, Sq, D)),
            "k_cache": _w((lambda *s: _rng.normal(s) * 0.8)(B, H, Sk, Dh)),
            "v_cache": _w((lambda *s: _rng.normal(s) * 0.05)(B, H, Sk, Dh)),
            "wq": _w((lambda *s: _rng.normal(s) * 0.8)(D, H * Dh) * (D ** -0.5)),
            "wo": _w((lambda *s: _rng.normal(s) * 0.05)(H * Dh, D) * ((H * Dh) ** -0.5)),
        }
    _B_in = _B_setup()

    return {
        "A_x": _A_in["x"],
        "A_k_cache": _A_in["k_cache"],
        "A_v_cache": _A_in["v_cache"],
        "A_wq": _A_in["wq"],
        "A_wo": _A_in["wo"],
        "B_x": _B_in["x"],
        "B_k_cache": _B_in["k_cache"],
        "B_v_cache": _B_in["v_cache"],
        "B_wq": _B_in["wq"],
        "B_wo": _B_in["wo"],
    }

def reference(A_x, A_k_cache, A_v_cache, A_wq, A_wo, B_x, B_k_cache, B_v_cache, B_wq, B_wo):
    def _A_ref(x, k_cache, v_cache, wq, wo):
        B, Sq, D = x.shape
        H, Dh = 32, 128
        q = (lambda x, *d: x.transpose(*d))((x @ wq).reshape(B, Sq, H, Dh), 0, 2, 1, 3)
        scores = jnp.einsum("bhqd,bhkd->bhqk", q, k_cache) * (Dh ** -0.5)
        p = _softmax(scores, axis=-1)
        o = jnp.einsum("bhqk,bhkd->bhqd", p, v_cache)
        return (lambda x, *d: x.transpose(*d))(o, 0, 2, 1, 3).reshape(B, Sq, H * Dh) @ wo

    def _B_ref(x, k_cache, v_cache, wq, wo):
        B, Sq, D = x.shape
        H, Dh = 32, 128
        q = (lambda x, *d: x.transpose(*d))((x @ wq).reshape(B, Sq, H, Dh), 0, 2, 1, 3)
        scores = jnp.einsum("bhqd,bhkd->bhqk", q, k_cache) * (Dh ** -0.5)
        p = _softmax(scores, axis=-1)
        o = jnp.einsum("bhqk,bhkd->bhqd", p, v_cache)
        return (lambda x, *d: x.transpose(*d))(o, 0, 2, 1, 3).reshape(B, Sq, H * Dh) @ wo

    a = _A_ref(A_x, A_k_cache, A_v_cache, A_wq, A_wo)
    b = _B_ref(B_x, B_k_cache, B_v_cache, B_wq, B_wo)
    return jnp.concatenate([a, b], axis=-1)
```

```python
import functools
import jax
import jax.numpy as jnp
import jax.experimental.pallas as pl
import jax.experimental.pallas.tpu as pltpu

B, SQ, D = 8, 144, 640
H, SK, DH = 32, 512, 128
SCALE = float(DH) ** -0.5


def _make(G):
    NHG = H // G
    GW = G * DH
    QP = D // B
    OP = GW // B

    def qk(q, k_ref, g):
        qh = q[:, g * DH:(g + 1) * DH]
        return jax.lax.dot_general(qh, k_ref[0, g], (((1,), (1,)), ((), ())),
                                   preferred_element_type=jnp.float32)

    def one_problem(x_ref, k_ref, v_ref, wq, wo, oall_ref):
        q = jnp.dot(x_ref[0], wq[...], preferred_element_type=jnp.float32)
        q = (q * SCALE).astype(jnp.bfloat16)
        s_next = qk(q, k_ref, 0)
        for g in range(G):
            s = s_next
            if g + 1 < G:
                s_next = qk(q, k_ref, g + 1)
            m = jnp.max(s, axis=-1, keepdims=True)
            p = jnp.exp(s - m)
            l = jnp.sum(p, axis=-1, keepdims=True)
            o = jnp.dot(p.astype(jnp.bfloat16), v_ref[0, g], preferred_element_type=jnp.float32)
            r = pl.reciprocal(l, approx=True)
            r = r * (2.0 - l * r)
            oall_ref[:, g * DH:(g + 1) * DH] = (o * r).astype(jnp.bfloat16)
        return jnp.dot(oall_ref[...], wo[...], preferred_element_type=jnp.float32)

    def kernel(ax, ak, av, awq, awo, bx, bk, bv, bwq, bwo, o_ref,
               oa_ref, ob_ref, acc_ref, wq_buf, wo_buf, sems):
        hg = pl.program_id(0)
        b = pl.program_id(1)
        slot = hg % 2

        def w_full(c, s):
            off = pl.multiple_of(c * GW, GW)
            return [
                pltpu.make_async_copy(awq.at[:, pl.ds(off, GW)], wq_buf.at[s, 0], sems.at[4 * s + 0]),
                pltpu.make_async_copy(awo.at[pl.ds(off, GW), :], wo_buf.at[s, 0], sems.at[4 * s + 1]),
                pltpu.make_async_copy(bwq.at[:, pl.ds(off, GW)], wq_buf.at[s, 1], sems.at[4 * s + 2]),
                pltpu.make_async_copy(bwo.at[pl.ds(off, GW), :], wo_buf.at[s, 1], sems.at[4 * s + 3]),
            ]

        def w_piece(c, s, i):
            off = pl.multiple_of(c * GW, GW)
            qr = pl.multiple_of(i * QP, QP)
            orow = pl.multiple_of(i * OP, OP)
            oroff = pl.multiple_of(c * GW + i * OP, OP)
            return [
                pltpu.make_async_copy(awq.at[pl.ds(qr, QP), pl.ds(off, GW)], wq_buf.at[s, 0, pl.ds(qr, QP)], sems.at[4 * s + 0]),
                pltpu.make_async_copy(awo.at[pl.ds(oroff, OP), :], wo_buf.at[s, 0, pl.ds(orow, OP)], sems.at[4 * s + 1]),
                pltpu.make_async_copy(bwq.at[pl.ds(qr, QP), pl.ds(off, GW)], wq_buf.at[s, 1, pl.ds(qr, QP)], sems.at[4 * s + 2]),
                pltpu.make_async_copy(bwo.at[pl.ds(oroff, OP), :], wo_buf.at[s, 1, pl.ds(orow, OP)], sems.at[4 * s + 3]),
            ]

        @pl.when(b == 0)
        def _():
            @pl.when(hg == 0)
            def _():
                for c in w_full(0, 0):
                    c.start()

            for c in w_full(hg, slot):
                c.wait()

        @pl.when(hg + 1 < NHG)
        def _():
            for c in w_piece(hg + 1, 1 - slot, b):
                c.start()

        first = hg == 0
        ca = one_problem(ax, ak, av, wq_buf.at[slot, 0], wo_buf.at[slot, 0], oa_ref)
        ta = jnp.where(first, ca, acc_ref[b, :, :D] + ca)
        acc_ref[b, :, :D] = ta
        cb = one_problem(bx, bk, bv, wq_buf.at[slot, 1], wo_buf.at[slot, 1], ob_ref)
        tb = jnp.where(first, cb, acc_ref[b, :, D:] + cb)
        acc_ref[b, :, D:] = tb

        @pl.when(hg == NHG - 1)
        def _():
            o_ref[0] = acc_ref[b].astype(o_ref.dtype)

    x_spec = pl.BlockSpec((1, SQ, D), lambda h, b: (b, 0, 0))
    kv_spec = pl.BlockSpec((1, G, SK, DH), lambda h, b: (b, h, 0, 0))
    w_spec = pl.BlockSpec(memory_space=pl.ANY)

    def fn(A_x, A_k_cache, A_v_cache, A_wq, A_wo, B_x, B_k_cache, B_v_cache, B_wq, B_wo):
        return pl.pallas_call(
            kernel,
            grid=(NHG, B),
            in_specs=[x_spec, kv_spec, kv_spec, w_spec, w_spec] * 2,
            out_specs=pl.BlockSpec((1, SQ, 2 * D), lambda h, b: (jnp.where(h == NHG - 1, b, 0), 0, 0)),
            out_shape=jax.ShapeDtypeStruct((B, SQ, 2 * D), jnp.bfloat16),
            scratch_shapes=[pltpu.VMEM((SQ, GW), jnp.bfloat16),
                            pltpu.VMEM((SQ, GW), jnp.bfloat16),
                            pltpu.VMEM((B, SQ, 2 * D), jnp.float32),
                            pltpu.VMEM((2, 2, D, GW), jnp.bfloat16),
                            pltpu.VMEM((2, 2, GW, D), jnp.bfloat16),
                            pltpu.SemaphoreType.DMA((8,))],
            compiler_params=pltpu.CompilerParams(
                dimension_semantics=("arbitrary", "arbitrary"),
                vmem_limit_bytes=100 * 1024 * 1024),
        )(A_x, A_k_cache, A_v_cache, A_wq, A_wo, B_x, B_k_cache, B_v_cache, B_wq, B_wo)

    return fn


_kernel_fn = _make(8)


@jax.jit
def pallas_concat_heads__mha_block_cached__mha_block_cached__near_ridge_kernel(
    A_x: jax.Array,
    A_k_cache: jax.Array,
    A_v_cache: jax.Array,
    A_wq: jax.Array,
    A_wo: jax.Array,
    B_x: jax.Array,
    B_k_cache: jax.Array,
    B_v_cache: jax.Array,
    B_wq: jax.Array,
    B_wo: jax.Array,
):
    return _kernel_fn(A_x, A_k_cache, A_v_cache, A_wq, A_wo,
                      B_x, B_k_cache, B_v_cache, B_wq, B_wo)
```

```python
import jax
import jax.numpy as jnp
import jax.experimental.pallas as pl
import jax.experimental.pallas.tpu as pltpu

B, SQ, D = 8, 144, 640
H, SK, DH = 32, 512, 128
SCALE = float(DH) ** -0.5

G = 8
NS = 4
NHG = H // G
GW = G * DH
NSTEPS = NHG * B


def _kernel(ax, ak, av, awq, awo, bx, bk, bv, bwq, bwo, o_ref,
            x_buf, q_buf, kv_buf, wq_buf, wo_buf, oall_ref, acc_ref,
            x_sem, kv_sem, w_sem):
    hg = pl.program_id(0)
    b = pl.program_id(1)
    t = hg * B + b
    slot = hg % 2
    xs, wqs, wos = (ax, bx), (awq, bwq), (awo, bwo)
    kvs = (ak, av, bk, bv)

    def x_copy(p):
        return pltpu.make_async_copy(xs[p], x_buf.at[p], x_sem.at[p])

    def wq_copy(p, c, s):
        off = pl.multiple_of(c * GW, GW)
        return pltpu.make_async_copy(wqs[p].at[:, pl.ds(off, GW)], wq_buf.at[s, p], w_sem.at[2 * s + p])

    def wo_copy(p, c):
        off = pl.multiple_of(c * GW, GW)
        return pltpu.make_async_copy(wos[p].at[pl.ds(off, GW), :], wo_buf.at[p], w_sem.at[4 + p])

    def kv_copies(tt):
        hh = tt // B
        bb = tt % B
        s = tt % NS
        h0 = pl.multiple_of(hh * G, G)
        return [pltpu.make_async_copy(src.at[bb, pl.ds(h0, G)], kv_buf.at[s, i], kv_sem.at[4 * s + i])
                for i, src in enumerate(kvs)]

    def qproj(p):
        w = wq_buf[slot, p]
        for bb in range(B):
            q = jnp.dot(x_buf[p, bb], w, preferred_element_type=jnp.float32)
            q_buf[p, bb] = (q * SCALE).astype(jnp.bfloat16)

    @pl.when(t == 0)
    def _():
        x_copy(0).start()
        wq_copy(0, 0, 0).start()

    @pl.when(b == 0)
    def _():
        @pl.when(hg == 0)
        def _():
            x_copy(0).wait()

        wq_copy(0, hg, slot).wait()

        @pl.when(hg == 0)
        def _():
            x_copy(1).start()
            wq_copy(1, 0, 0).start()
            for c in kv_copies(0):
                c.start()
            wo_copy(0, 0).start()
            wo_copy(1, 0).start()

        @pl.when(hg > 0)
        def _():
            for p in range(2):
                wo_copy(p, hg).start()

            @pl.when(hg + 1 < NHG)
            def _():
                for p in range(2):
                    wq_copy(p, hg + 1, 1 - slot).start()

        qproj(0)

        @pl.when(hg == 0)
        def _():
            x_copy(1).wait()
            for c in kv_copies(1):
                c.start()

        wq_copy(1, hg, slot).wait()
        qproj(1)

        @pl.when(hg == 0)
        def _():
            for tt in range(2, NS - 1):
                for c in kv_copies(tt):
                    c.start()
            for p in range(2):
                wq_copy(p, 1, 1).start()

        wo_copy(0, hg).wait()
        wo_copy(1, hg).wait()

    for c in kv_copies(t):
        c.wait()

    s_kv = t % NS

    def attn(p):
        k_ref = kv_buf.at[s_kv, 2 * p]
        v_ref = kv_buf.at[s_kv, 2 * p + 1]
        q_ref = q_buf.at[p, b]

        def qk(g):
            return jax.lax.dot_general(q_ref[:, g * DH:(g + 1) * DH], k_ref[g],
                                       (((1,), (1,)), ((), ())),
                                       preferred_element_type=jnp.float32)

        s_next = qk(0)
        for g in range(G):
            s = s_next
            if g + 1 < G:
                s_next = qk(g + 1)
            m = jnp.max(s, axis=-1, keepdims=True)
            pr = jnp.exp(s - m)
            l = jnp.sum(pr, axis=-1, keepdims=True)
            o = jnp.dot(pr.astype(jnp.bfloat16), v_ref[g], preferred_element_type=jnp.float32)
            r = pl.reciprocal(l, approx=True)
            r = r * (2.0 - l * r)
            oall_ref[p, :, g * DH:(g + 1) * DH] = (o * r).astype(jnp.bfloat16)
        return jnp.dot(oall_ref[p], wo_buf[p], preferred_element_type=jnp.float32)

    first = hg == 0
    ca = attn(0)
    acc_ref[b, :, :D] = jnp.where(first, ca, acc_ref[b, :, :D] + ca)
    cb = attn(1)
    acc_ref[b, :, D:] = jnp.where(first, cb, acc_ref[b, :, D:] + cb)

    @pl.when(t + NS - 1 < NSTEPS)
    def _():
        for c in kv_copies(t + NS - 1):
            c.start()

    @pl.when(hg == NHG - 1)
    def _():
        o_ref[0] = acc_ref[b].astype(o_ref.dtype)


@jax.jit
def pallas_concat_heads__mha_block_cached__mha_block_cached__near_ridge_kernel(
    A_x: jax.Array,
    A_k_cache: jax.Array,
    A_v_cache: jax.Array,
    A_wq: jax.Array,
    A_wo: jax.Array,
    B_x: jax.Array,
    B_k_cache: jax.Array,
    B_v_cache: jax.Array,
    B_wq: jax.Array,
    B_wo: jax.Array,
):
    any_spec = pl.BlockSpec(memory_space=pl.ANY)
    return pl.pallas_call(
        _kernel,
        grid=(NHG, B),
        in_specs=[any_spec] * 10,
        out_specs=pl.BlockSpec((1, SQ, 2 * D), lambda h, b: (jnp.where(h == NHG - 1, b, 0), 0, 0)),
        out_shape=jax.ShapeDtypeStruct((B, SQ, 2 * D), jnp.bfloat16),
        scratch_shapes=[
            pltpu.VMEM((2, B, SQ, D), jnp.bfloat16),
            pltpu.VMEM((2, B, SQ, GW), jnp.bfloat16),
            pltpu.VMEM((NS, 4, G, SK, DH), jnp.bfloat16),
            pltpu.VMEM((2, 2, D, GW), jnp.bfloat16),
            pltpu.VMEM((2, GW, D), jnp.bfloat16),
            pltpu.VMEM((2, SQ, GW), jnp.bfloat16),
            pltpu.VMEM((B, SQ, 2 * D), jnp.float32),
            pltpu.SemaphoreType.DMA((2,)),
            pltpu.SemaphoreType.DMA((4 * NS,)),
            pltpu.SemaphoreType.DMA((6,)),
        ],
        compiler_params=pltpu.CompilerParams(
            dimension_semantics=("arbitrary", "arbitrary"),
            vmem_limit_bytes=100 * 1024 * 1024),
    )(A_x, A_k_cache, A_v_cache, A_wq, A_wo, B_x, B_k_cache, B_v_cache, B_wq, B_wo)
```

```python
import jax
import jax.numpy as jnp
import jax.experimental.pallas as pl
import jax.experimental.pallas.tpu as pltpu

B, SQ, D = 8, 144, 640
H, SK, DH = 32, 512, 128
SCALE_BF16 = 0.08837890625

G = 8
NS = 4
NHG = H // G
GW = G * DH
NSTEPS = NHG * B


def _kernel(ax, ak, av, awq, awo, bx, bk, bv, bwq, bwo, o_ref,
            x_buf, q_buf, kv_buf, wq_buf, wo_buf, oall_ref, acc_ref,
            x_sem, kv_sem, w_sem):
    hg = pl.program_id(0)
    b = pl.program_id(1)
    t = hg * B + b
    slot = hg % 2
    xs, wqs, wos = (ax, bx), (awq, bwq), (awo, bwo)
    kvs = (ak, av, bk, bv)

    def x_copy(p):
        return pltpu.make_async_copy(xs[p], x_buf.at[p], x_sem.at[p])

    def wq_copy(p, c, s):
        off = pl.multiple_of(c * GW, GW)
        return pltpu.make_async_copy(wqs[p].at[:, pl.ds(off, GW)], wq_buf.at[s, p], w_sem.at[2 * s + p])

    def wo_copy(p, c):
        off = pl.multiple_of(c * GW, GW)
        return pltpu.make_async_copy(wos[p].at[pl.ds(off, GW), :], wo_buf.at[p], w_sem.at[4 + p])

    def kv_copies(tt):
        hh = tt // B
        bb = tt % B
        s = tt % NS
        h0 = pl.multiple_of(hh * G, G)
        return [pltpu.make_async_copy(src.at[bb, pl.ds(h0, G)], kv_buf.at[s, i], kv_sem.at[4 * s + i])
                for i, src in enumerate(kvs)]

    def qproj(p):
        w = wq_buf[slot, p]
        for bb in range(B):
            q = jnp.dot(x_buf[p, bb], w, preferred_element_type=jnp.float32)
            q_buf[p, bb] = q.astype(jnp.bfloat16)

    @pl.when(t == 0)
    def _():
        x_copy(0).start()
        wq_copy(0, 0, 0).start()

    @pl.when(b == 0)
    def _():
        @pl.when(hg == 0)
        def _():
            x_copy(0).wait()

        wq_copy(0, hg, slot).wait()

        @pl.when(hg == 0)
        def _():
            x_copy(1).start()
            wq_copy(1, 0, 0).start()
            for c in kv_copies(0):
                c.start()
            wo_copy(0, 0).start()
            wo_copy(1, 0).start()

        @pl.when(hg > 0)
        def _():
            for p in range(2):
                wo_copy(p, hg).start()

            @pl.when(hg + 1 < NHG)
            def _():
                for p in range(2):
                    wq_copy(p, hg + 1, 1 - slot).start()

        qproj(0)

        @pl.when(hg == 0)
        def _():
            x_copy(1).wait()
            for c in kv_copies(1):
                c.start()

        wq_copy(1, hg, slot).wait()
        qproj(1)

        @pl.when(hg == 0)
        def _():
            for tt in range(2, NS - 1):
                for c in kv_copies(tt):
                    c.start()
            for p in range(2):
                wq_copy(p, 1, 1).start()

        wo_copy(0, hg).wait()
        wo_copy(1, hg).wait()

    for c in kv_copies(t):
        c.wait()

    s_kv = t % NS

    def attn(p):
        k_ref = kv_buf.at[s_kv, 2 * p]
        v_ref = kv_buf.at[s_kv, 2 * p + 1]
        q_ref = q_buf.at[p, b]

        def qk(g):
            return jax.lax.dot_general(q_ref[:, g * DH:(g + 1) * DH], k_ref[g],
                                       (((1,), (1,)), ((), ())),
                                       preferred_element_type=jnp.float32)

        s_next = qk(0)
        for g in range(G):
            s = s_next
            if g + 1 < G:
                s_next = qk(g + 1)
            s = s.astype(jnp.bfloat16).astype(jnp.float32)
            s = (s * SCALE_BF16).astype(jnp.bfloat16).astype(jnp.float32)
            m = jnp.max(s, axis=-1, keepdims=True)
            pr = jnp.exp(s - m)
            l = jnp.sum(pr, axis=-1, keepdims=True)
            o = jnp.dot(pr.astype(jnp.bfloat16), v_ref[g], preferred_element_type=jnp.float32)
            r = pl.reciprocal(l, approx=True)
            r = r * (2.0 - l * r)
            oall_ref[p, :, g * DH:(g + 1) * DH] = (o * r).astype(jnp.bfloat16)
        return jnp.dot(oall_ref[p], wo_buf[p], preferred_element_type=jnp.float32)

    first = hg == 0
    ca = attn(0)
    acc_ref[b, :, :D] = jnp.where(first, ca, acc_ref[b, :, :D] + ca)
    cb = attn(1)
    acc_ref[b, :, D:] = jnp.where(first, cb, acc_ref[b, :, D:] + cb)

    @pl.when(t + NS - 1 < NSTEPS)
    def _():
        for c in kv_copies(t + NS - 1):
            c.start()

    @pl.when(hg == NHG - 1)
    def _():
        o_ref[0] = acc_ref[b].astype(o_ref.dtype)


@jax.jit
def pallas_concat_heads__mha_block_cached__mha_block_cached__near_ridge_kernel(
    A_x: jax.Array,
    A_k_cache: jax.Array,
    A_v_cache: jax.Array,
    A_wq: jax.Array,
    A_wo: jax.Array,
    B_x: jax.Array,
    B_k_cache: jax.Array,
    B_v_cache: jax.Array,
    B_wq: jax.Array,
    B_wo: jax.Array,
):
    any_spec = pl.BlockSpec(memory_space=pl.ANY)
    return pl.pallas_call(
        _kernel,
        grid=(NHG, B),
        in_specs=[any_spec] * 10,
        out_specs=pl.BlockSpec((1, SQ, 2 * D), lambda h, b: (jnp.where(h == NHG - 1, b, 0), 0, 0)),
        out_shape=jax.ShapeDtypeStruct((B, SQ, 2 * D), jnp.bfloat16),
        scratch_shapes=[
            pltpu.VMEM((2, B, SQ, D), jnp.bfloat16),
            pltpu.VMEM((2, B, SQ, GW), jnp.bfloat16),
            pltpu.VMEM((NS, 4, G, SK, DH), jnp.bfloat16),
            pltpu.VMEM((2, 2, D, GW), jnp.bfloat16),
            pltpu.VMEM((2, GW, D), jnp.bfloat16),
            pltpu.VMEM((2, SQ, GW), jnp.bfloat16),
            pltpu.VMEM((B, SQ, 2 * D), jnp.float32),
            pltpu.SemaphoreType.DMA((2,)),
            pltpu.SemaphoreType.DMA((4 * NS,)),
            pltpu.SemaphoreType.DMA((6,)),
        ],
        compiler_params=pltpu.CompilerParams(
            dimension_semantics=("arbitrary", "arbitrary"),
            vmem_limit_bytes=100 * 1024 * 1024),
    )(A_x, A_k_cache, A_v_cache, A_wq, A_wo, B_x, B_k_cache, B_v_cache, B_wq, B_wo)
```

```python
import jax
import jax.numpy as jnp
import jax.experimental.pallas as pl
import jax.experimental.pallas.tpu as pltpu

B, SQ, D = 8, 144, 640
H, SK, DH = 32, 512, 128
SCALE_BF16 = 0.08837890625

G = 8
LA = 2
NS = 4
NHG = H // G
GW = G * DH
NSTEPS = NHG * B


def _kernel(ax, ak, av, awq, awo, bx, bk, bv, bwq, bwo, o_ref,
            x_buf, q_buf, kv_buf, wq_buf, wo_buf, oall_ref, acc_ref,
            x_sem, kv_sem, w_sem):
    hg = pl.program_id(0)
    b = pl.program_id(1)
    t = hg * B + b
    slot = hg % 2
    xs, wqs, wos = (ax, bx), (awq, bwq), (awo, bwo)
    kvs = (ak, av, bk, bv)

    def x_copy(p):
        return pltpu.make_async_copy(xs[p], x_buf.at[p], x_sem.at[p])

    def wq_copy(p, c, s):
        off = pl.multiple_of(c * GW, GW)
        return pltpu.make_async_copy(wqs[p].at[:, pl.ds(off, GW)], wq_buf.at[s, p], w_sem.at[2 * s + p])

    def wo_copy(p, c):
        off = pl.multiple_of(c * GW, GW)
        return pltpu.make_async_copy(wos[p].at[pl.ds(off, GW), :], wo_buf.at[p], w_sem.at[4 + p])

    def kv_copies(tt):
        hh = tt // B
        bb = tt % B
        s = tt % NS
        h0 = pl.multiple_of(hh * G, G)
        return [pltpu.make_async_copy(src.at[bb, pl.ds(h0, G)], kv_buf.at[s, i], kv_sem.at[4 * s + i])
                for i, src in enumerate(kvs)]

    def qproj(p):
        w = wq_buf[slot, p]
        for bb in range(B):
            q = jnp.dot(x_buf[p, bb], w, preferred_element_type=jnp.float32)
            q_buf[p, bb] = q.astype(jnp.bfloat16)

    @pl.when(t == 0)
    def _():
        x_copy(0).start()
        wq_copy(0, 0, 0).start()

    @pl.when(b == 0)
    def _():
        @pl.when(hg == 0)
        def _():
            x_copy(0).wait()

        wq_copy(0, hg, slot).wait()

        @pl.when(hg == 0)
        def _():
            x_copy(1).start()
            wq_copy(1, 0, 0).start()
            for c in kv_copies(0):
                c.start()
            wo_copy(0, 0).start()
            wo_copy(1, 0).start()

        @pl.when(hg > 0)
        def _():
            for p in range(2):
                wo_copy(p, hg).start()

            @pl.when(hg + 1 < NHG)
            def _():
                for p in range(2):
                    wq_copy(p, hg + 1, 1 - slot).start()

        qproj(0)

        @pl.when(hg == 0)
        def _():
            x_copy(1).wait()
            for c in kv_copies(1):
                c.start()

        wq_copy(1, hg, slot).wait()
        qproj(1)

        @pl.when(hg == 0)
        def _():
            for tt in range(2, NS - 1):
                for c in kv_copies(tt):
                    c.start()
            for p in range(2):
                wq_copy(p, 1, 1).start()

        wo_copy(0, hg).wait()
        wo_copy(1, hg).wait()

    for c in kv_copies(t):
        c.wait()

    s_kv = t % NS

    def attn(p):
        k_ref = kv_buf.at[s_kv, 2 * p]
        v_ref = kv_buf.at[s_kv, 2 * p + 1]
        q_ref = q_buf.at[p, b]

        def qk(g):
            return jax.lax.dot_general(q_ref[:, g * DH:(g + 1) * DH], k_ref[g],
                                       (((1,), (1,)), ((), ())),
                                       preferred_element_type=jnp.float32)

        pending = [qk(g) for g in range(LA)]
        for g in range(G):
            s = pending.pop(0)
            if g + LA < G:
                pending.append(qk(g + LA))
            s = s.astype(jnp.bfloat16).astype(jnp.float32)
            s = (s * SCALE_BF16).astype(jnp.bfloat16).astype(jnp.float32)
            m = jnp.max(s, axis=-1, keepdims=True)
            pr = jnp.exp(s - m)
            l = jnp.sum(pr, axis=-1, keepdims=True)
            o = jnp.dot(pr.astype(jnp.bfloat16), v_ref[g], preferred_element_type=jnp.float32)
            r = pl.reciprocal(l, approx=True)
            r = r * (2.0 - l * r)
            oall_ref[p, :, g * DH:(g + 1) * DH] = (o * r).astype(jnp.bfloat16)
        return jnp.dot(oall_ref[p], wo_buf[p], preferred_element_type=jnp.float32)

    first = hg == 0
    ca = attn(0)
    acc_ref[b, :, :D] = jnp.where(first, ca, acc_ref[b, :, :D] + ca)
    cb = attn(1)
    acc_ref[b, :, D:] = jnp.where(first, cb, acc_ref[b, :, D:] + cb)

    @pl.when(t + NS - 1 < NSTEPS)
    def _():
        for c in kv_copies(t + NS - 1):
            c.start()

    @pl.when(hg == NHG - 1)
    def _():
        o_ref[0] = acc_ref[b].astype(o_ref.dtype)


@jax.jit
def pallas_concat_heads__mha_block_cached__mha_block_cached__near_ridge_kernel(
    A_x: jax.Array,
    A_k_cache: jax.Array,
    A_v_cache: jax.Array,
    A_wq: jax.Array,
    A_wo: jax.Array,
    B_x: jax.Array,
    B_k_cache: jax.Array,
    B_v_cache: jax.Array,
    B_wq: jax.Array,
    B_wo: jax.Array,
):
    any_spec = pl.BlockSpec(memory_space=pl.ANY)
    return pl.pallas_call(
        _kernel,
        grid=(NHG, B),
        in_specs=[any_spec] * 10,
        out_specs=pl.BlockSpec((1, SQ, 2 * D), lambda h, b: (jnp.where(h == NHG - 1, b, 0), 0, 0)),
        out_shape=jax.ShapeDtypeStruct((B, SQ, 2 * D), jnp.bfloat16),
        scratch_shapes=[
            pltpu.VMEM((2, B, SQ, D), jnp.bfloat16),
            pltpu.VMEM((2, B, SQ, GW), jnp.bfloat16),
            pltpu.VMEM((NS, 4, G, SK, DH), jnp.bfloat16),
            pltpu.VMEM((2, 2, D, GW), jnp.bfloat16),
            pltpu.VMEM((2, GW, D), jnp.bfloat16),
            pltpu.VMEM((2, SQ, GW), jnp.bfloat16),
            pltpu.VMEM((B, SQ, 2 * D), jnp.float32),
            pltpu.SemaphoreType.DMA((2,)),
            pltpu.SemaphoreType.DMA((4 * NS,)),
            pltpu.SemaphoreType.DMA((6,)),
        ],
        compiler_params=pltpu.CompilerParams(
            dimension_semantics=("arbitrary", "arbitrary"),
            vmem_limit_bytes=100 * 1024 * 1024),
    )(A_x, A_k_cache, A_v_cache, A_wq, A_wo, B_x, B_k_cache, B_v_cache, B_wq, B_wo)
```
